```python
import os as _os
_os.environ.setdefault("JAX_PLATFORMS", "cpu")
import jax
import jax.numpy as jnp

def _softmax(x, axis=-1):
    return jax.nn.softmax(x, axis=axis)
def _gelu(x):
    return jax.nn.gelu(x, approximate=True)
def _silu(x):
    return jax.nn.silu(x)
def _sigmoid(x):
    return jax.nn.sigmoid(x)
def _layernorm(x, axis=-1, eps=1e-5):
    m = jnp.mean(x, axis=axis, keepdims=True)
    v = jnp.var(x, axis=axis, keepdims=True)
    return (x - m) / jnp.sqrt(v + eps)
def _scatter_add(tgt, idx, src, axis=0):
    return tgt.at[idx].add(src)
def _segment_sum(src, seg, n):
    return jax.ops.segment_sum(src, seg, n)
class _Rng:
    def __init__(self, key):
        self._k = key
    def _next(self):
        self._k, sub = jax.random.split(self._k)
        return sub
    def normal(self, shape):
        return jax.random.normal(self._next(), shape, dtype=jnp.bfloat16)
    def randint(self, lo, hi, shape):
        return jax.random.randint(self._next(), shape, lo, hi, dtype=jnp.int32)
    def uniform(self, shape, lo=0.0, hi=1.0):
        return jax.random.uniform(self._next(), shape, jnp.bfloat16, lo, hi)
    def permutation(self, n):
        return jax.random.permutation(self._next(), n)


kernel_name = 'standalone__instancenorm__sampling'

def setup_inputs():
    _rng = _Rng(jax.random.key(int.from_bytes(__import__("os").urandom(4), "little")))
    _w = (lambda a: (lambda t: t.astype(jnp.bfloat16) if jnp.issubdtype(t.dtype, jnp.floating) else t)(jnp.asarray(a)))
    B, C, H, W = 16, 640, 16, 32
    return {
        "x": _w((lambda *s: _rng.normal(s) * 0.05)(B, C, H, W)),
        "g": _w((lambda *s: _rng.normal(s) * 0.05)(C) + 1.0),
        "b": _w((lambda *s: _rng.normal(s) * 0.05)(C)),
    }

def reference(x, g, b):
    mu = x.mean(axis=(-2, -1), keepdims=True)
    var = ((x - mu) * (x - mu)).mean(axis=(-2, -1), keepdims=True)
    xhat = (x - mu) / jnp.sqrt(var + 1e-5)
    return xhat * g.reshape(1, -1, 1, 1) + b.reshape(1, -1, 1, 1)
```

```python
import jax
import jax.numpy as jnp
import jax.experimental.pallas as pl
import jax.experimental.pallas.tpu as pltpu

_EPS = 1e-5


@jax.jit
def pallas_standalone__instancenorm__sampling_kernel(
    x: jax.Array,
    g: jax.Array,
    b: jax.Array,
):
    B, C, H, W = x.shape
    S = H * W
    K = B // 2
    GR = 2 * S
    WROWS = 16
    TAIL = 320

    def kernel(x_hbm, g_hbm, b_hbm, o_hbm, buf, gv, bv, sems):
        cg = pltpu.make_async_copy(g_hbm, gv, sems.at[0])
        cb = pltpu.make_async_copy(b_hbm, bv, sems.at[0])
        r0 = pltpu.make_async_copy(
            x_hbm.at[:, pl.ds(0, S), :], buf.at[:, pl.ds(0, S), :], sems.at[0])
        r1a = pltpu.make_async_copy(
            x_hbm.at[pl.ds(0, K - 1), pl.ds(S, S), :],
            buf.at[pl.ds(0, K - 1), pl.ds(S, S), :], sems.at[1])
        r1b = pltpu.make_async_copy(
            x_hbm.at[K - 1, pl.ds(S, S - TAIL), :],
            buf.at[K - 1, pl.ds(S, S - TAIL), :], sems.at[1])
        r2 = pltpu.make_async_copy(
            x_hbm.at[K - 1, pl.ds(GR - TAIL, TAIL), :],
            buf.at[K - 1, pl.ds(GR - TAIL, TAIL), :], sems.at[2])
        cg.start()
        cb.start()
        r0.start(priority=1)
        r1a.start(priority=1)
        r1b.start(priority=1)
        r2.start(priority=1)
        cg.wait()
        cb.wait()
        r0.wait()
        gf = gv[...].astype(jnp.float32).reshape(1, C)
        bf = bv[...].astype(jnp.float32).reshape(1, C)

        def normalize(k, s):
            xv = buf[k, pl.ds(s * S, S), :].astype(jnp.float32)
            mu = jnp.mean(xv, axis=0, keepdims=True)
            xc = xv - mu
            var = jnp.mean(xc * xc, axis=0, keepdims=True)
            inv = jax.lax.rsqrt(var + _EPS)
            buf[k, pl.ds(s * S, S), :] = (xc * (inv * gf) + bf).astype(buf.dtype)

        def normalize_range(k0, k1, s):
            def body(k, carry):
                normalize(k, s)
                return carry
            jax.lax.fori_loop(k0, k1, body, 0)

        def write_out(row0):
            for j in range(S // WROWS):
                st = row0 + j * WROWS
                pltpu.make_async_copy(
                    buf.at[:, pl.ds(st, WROWS), :],
                    o_hbm.at[:, pl.ds(st, WROWS), :], sems.at[0]).start()

        normalize_range(0, K, 0)
        r1a.wait()
        r1b.wait()
        write_out(0)
        normalize_range(0, K - 1, 1)
        r2.wait()
        normalize(K - 1, 1)
        write_out(S)
        pltpu.make_async_copy(buf, o_hbm, sems.at[0]).wait()

    xt = x.transpose(0, 2, 3, 1).reshape(K, GR, C)
    out = pl.pallas_call(
        kernel,
        in_specs=[pl.BlockSpec(memory_space=pl.ANY)] * 3,
        out_specs=pl.BlockSpec(memory_space=pl.ANY),
        out_shape=jax.ShapeDtypeStruct((K, GR, C), x.dtype),
        scratch_shapes=[
            pltpu.VMEM((K, GR, C), x.dtype),
            pltpu.VMEM((C,), g.dtype),
            pltpu.VMEM((C,), b.dtype),
            pltpu.SemaphoreType.DMA((3,)),
        ],
        compiler_params=pltpu.CompilerParams(vmem_limit_bytes=64 * 1024 * 1024),
    )(xt, g, b)
    return out.reshape(B, H, W, C).transpose(0, 3, 1, 2)
```
